```python
import os as _os
_os.environ.setdefault("JAX_PLATFORMS", "cpu")
import jax
import jax.numpy as jnp

def _softmax(x, axis=-1):
    return jax.nn.softmax(x, axis=axis)
def _gelu(x):
    return jax.nn.gelu(x, approximate=True)
def _silu(x):
    return jax.nn.silu(x)
def _sigmoid(x):
    return jax.nn.sigmoid(x)
def _layernorm(x, axis=-1, eps=1e-5):
    m = jnp.mean(x, axis=axis, keepdims=True)
    v = jnp.var(x, axis=axis, keepdims=True)
    return (x - m) / jnp.sqrt(v + eps)
def _scatter_add(tgt, idx, src, axis=0):
    return tgt.at[idx].add(src)
def _segment_sum(src, seg, n):
    return jax.ops.segment_sum(src, seg, n)
class _Rng:
    def __init__(self, key):
        self._k = key
    def _next(self):
        self._k, sub = jax.random.split(self._k)
        return sub
    def normal(self, shape):
        return jax.random.normal(self._next(), shape, dtype=jnp.bfloat16)
    def randint(self, lo, hi, shape):
        return jax.random.randint(self._next(), shape, lo, hi, dtype=jnp.int32)
    def uniform(self, shape, lo=0.0, hi=1.0):
        return jax.random.uniform(self._next(), shape, jnp.bfloat16, lo, hi)
    def permutation(self, n):
        return jax.random.permutation(self._next(), n)


kernel_name = 'gated_mix__mha_block__softmax_full_mha__prompt'

def setup_inputs():
    _rng = _Rng(jax.random.key(int.from_bytes(__import__("os").urandom(4), "little")))
    _w = (lambda a: (lambda t: t.astype(jnp.bfloat16) if jnp.issubdtype(t.dtype, jnp.floating) else t)(jnp.asarray(a)))
    def _A_setup():
        B, S, D, H = 1, 2048, 448, 16
        return {
            "x": _w((lambda *s: _rng.normal(s) * 0.05)(B, S, D)),
            "wqkv": _w((lambda *s: _rng.normal(s) * 0.4)(D, 3 * D)),
            "wo": _w((lambda *s: _rng.normal(s) * 0.05)(D, D)),
        }
    _A_in = _A_setup()

    def _B_setup():
        B, S, D = 1, 2048, 448
        return {
            "x": _w((lambda *s: _rng.normal(s) * 0.05)(B, S, D)),
            "wqkv": _w((lambda *s: _rng.normal(s) * 0.4)(D, 3 * D)),
            "wo": _w((lambda *s: _rng.normal(s) * 0.05)(D, D)),
        }
    _B_in = _B_setup()

    return {
        "A_x": _A_in["x"],
        "A_wqkv": _A_in["wqkv"],
        "A_wo": _A_in["wo"],
        "B_x": _B_in["x"],
        "B_wqkv": _B_in["wqkv"],
        "B_wo": _B_in["wo"],
        "gate_w": _w((lambda *s: _rng.normal(s) * 0.05)(448) * 16.0),
    }

def reference(A_x, A_wqkv, A_wo, B_x, B_wqkv, B_wo, gate_w):
    def _A_ref(x, wqkv, wo):
        B, S, D = x.shape
        H = 16
        Dh = D // H
        qkv = (lambda x, *d: x.transpose(*d))((x @ wqkv).reshape(B, S, 3, H, Dh), 2, 0, 3, 1, 4)
        q, k, v = qkv[0], qkv[1], qkv[2]
        scores = jnp.einsum("bhqd,bhkd->bhqk", q, k) * (Dh ** -0.5)
        p = _softmax(scores, axis=-1)
        o = jnp.einsum("bhqk,bhkd->bhqd", p, v)
        return (lambda x, *d: x.transpose(*d))(o, 0, 2, 1, 3).reshape(B, S, D) @ wo

    def _B_ref(x, wqkv, wo):
        B, S, D = x.shape
        H = 16; Dh = D // H
        qkv = (lambda x, *d: x.transpose(*d))((x @ wqkv).reshape(B, S, 3, H, Dh), 2, 0, 3, 1, 4)
        q, k, v = qkv[0], qkv[1], qkv[2]
        scale = Dh ** -0.5
        scores = jnp.einsum("bhqd,bhkd->bhqk", q, k) * scale
        p = _softmax(scores, axis=-1)
        o = jnp.einsum("bhqk,bhkd->bhqd", p, v)
        return (lambda x, *d: x.transpose(*d))(o, 0, 2, 1, 3).reshape(B, S, D) @ wo

    x = A_x
    g = _sigmoid((x * gate_w).sum(-1, keepdims=True))
    a = _A_ref(x, A_wqkv, A_wo)
    b = _B_ref(x, B_wqkv, B_wo)
    return g * a + (1 - g) * b
```

```python
import functools, math
import jax
import jax.numpy as jnp
import numpy as np
from jax import lax
import jax.experimental.pallas as pl
import jax.experimental.pallas.tpu as pltpu

S, D, H, DH = 2048, 448, 16, 28
HP = 32
DP = H * HP
f32 = jnp.float32; bf16 = jnp.bfloat16
INTERP = False

def mm(a, b):
    if INTERP:
        a = a.astype(f32); b = b.astype(f32)
    return lax.dot_general(a, b, (((1,), (0,)), ((), ())), preferred_element_type=f32)

def _pad_rows(wt, dst_ref, n_heads, row0=0):
    for j in range(n_heads):
        dst_ref[row0 + HP*j: row0 + HP*j + DH, :] = wt[DH*j: DH*j + DH, :]
        dst_ref[row0 + HP*j + DH: row0 + HP*(j+1), :] = jnp.zeros((HP-DH, wt.shape[1]), wt.dtype)

def make_kernel(BQ=1024, CK=256, NITER=None, DEP=1):
    NQ = S // BQ
    NT = 2 * H * NQ
    def kernel(x_ref, wqkva_ref, woa_ref, wqkvb_ref, wob_ref, gw_ref, o_ref,
               wpad_s, k_s, qt_s, vt_s, ot_s, wot_s, s0_s, s1_s):
        c = (DH ** -0.5) * math.log2(math.e)
        gw = jnp.broadcast_to(gw_ref[...], (16, D))
        gl = mm(gw, x_ref[...])[0:1, :]
        g = jax.nn.sigmoid(gl)

        for blk, (wqkv_ref, wo_ref) in enumerate(((wqkva_ref, woa_ref), (wqkvb_ref, wob_ref))):
            wt = wqkv_ref[...].astype(f32).T
            _pad_rows(wt, wpad_s, 3*H)
            wq = wpad_s[0:DP, :].astype(bf16)
            wk = wpad_s[DP:2*DP, :].astype(bf16)
            wv = wpad_s[2*DP:3*DP, :].astype(bf16)
            xt = x_ref[...]
            qt = mm(wq, xt) * c
            for gidx in range(4):
                for i in range(NQ):
                    qt_s[(blk*4+gidx)*NQ + i] = qt[128*gidx:128*gidx+128, BQ*i:BQ*(i+1)].astype(bf16)
            kt = mm(wk, xt)
            for gidx in range(4):
                k_s[blk*4+gidx] = kt[128*gidx:128*gidx+128, :].T.astype(bf16)
            vt = mm(wv, xt)
            row = lax.broadcasted_iota(jnp.int32, (DP, S), 0)
            vt = jnp.where(row % HP == DH, 1.0, vt)
            vt_s[blk*H:(blk+1)*H] = vt.astype(bf16).reshape(H, HP, S)
            _pad_rows(wo_ref[...].astype(f32), wpad_s, H)
            wot_s[blk] = wpad_s[0:DP, :].T.astype(bf16)

        def qmask(t):
            h = t // NQ
            i = t % NQ
            gidx = h // 4
            j = h % 4
            qg = qt_s[gidx*NQ + i]
            r = lax.broadcasted_iota(jnp.int32, (128, BQ), 0)
            return gidx, jnp.where((r >= j*HP) & (r < j*HP + HP), qg, jnp.zeros_like(qg))

        NC = S // CK
        def step(t_cur, s_cur, m_cur, t_nxt, s_nxt):
            macc = None
            o = None
            ties = []
            if t_nxt is not None:
                gidx, qm = qmask(t_nxt)
            if t_cur is not None:
                h = t_cur // NQ
                i = t_cur % NQ
            for c in range(NC):
                sl = slice(c*CK, (c+1)*CK)
                if t_nxt is not None:
                    s = mm(k_s[gidx, sl, :], qm)
                    s_nxt[sl, :] = s
                    mx = jnp.max(s.reshape(CK//8, 8, BQ), axis=0)
                    macc = mx if macc is None else jnp.maximum(macc, mx)
                if t_cur is not None:
                    m_eff = m_cur
                    if t_nxt is not None and DEP:
                        src_v = mx if DEP == 1 else (ties[-1] if ties else None)
                        if src_v is not None:
                            z = lax.bitcast_convert_type(src_v[0:1, :], jnp.uint32)
                            z = lax.shift_right_logical(lax.shift_right_logical(z, jnp.uint32(31)), jnp.uint32(1))
                            m_eff = lax.bitcast_convert_type(lax.bitcast_convert_type(m_cur, jnp.uint32) | z, f32)
                        ties.append(mx)
                    p = jnp.exp2(s_cur[sl, :] - m_eff).astype(bf16)
                    oc = mm(vt_s[h, :, sl], p)
                    o = oc if o is None else o + oc
            if t_cur is not None:
                ot_s[i, pl.ds(pl.multiple_of(h*HP, HP), HP), :] = o
            if t_nxt is not None:
                return jnp.max(macc, axis=0, keepdims=True)

        m0 = step(None, None, None, 0, s0_s)
        def body(u, m):
            t = 2*u
            m1 = step(t, s0_s, m, t+1, s1_s)
            m2 = step(t+1, s1_s, m1, jnp.minimum(t+2, NT-1), s0_s)
            return m2
        lax.fori_loop(0, NITER or NT//2, body, m0)

        for i in range(NQ):
            acc = None
            for blk in range(2):
                gate = g if blk == 0 else 1.0 - g
                o = ot_s[i, blk*DP:(blk+1)*DP, :]
                o = o.reshape(H, HP, BQ)
                l = o[:, DH:DH+1, :]
                on = (o * (gate[:, BQ*i:BQ*(i+1)].reshape(1, 1, BQ) / l)).reshape(DP, BQ).astype(bf16)
                y = mm(wot_s[blk], on)
                acc = y if acc is None else acc + y
            o_ref[:, BQ*i:BQ*(i+1)] = acc.astype(o_ref.dtype)
    return kernel


BQ = 1024
CK = 128


@jax.jit
def pallas_gated_mix__mha_block__softmax_full_mha__prompt_kernel(
    A_x: jax.Array,
    A_wqkv: jax.Array,
    A_wo: jax.Array,
    B_x: jax.Array,
    B_wqkv: jax.Array,
    B_wo: jax.Array,
    gate_w: jax.Array,
):
    del B_x
    NQ = S // BQ
    out = pl.pallas_call(
        make_kernel(BQ, CK, None, 2),
        out_shape=jax.ShapeDtypeStruct((D, S), jnp.bfloat16),
        scratch_shapes=[
            pltpu.VMEM((3*DP, D), jnp.float32),
            pltpu.VMEM((8, S, 128), jnp.bfloat16),
            pltpu.VMEM((8*NQ, 128, BQ), jnp.bfloat16),
            pltpu.VMEM((2*H, HP, S), jnp.bfloat16),
            pltpu.VMEM((NQ, 2*DP, BQ), jnp.float32),
            pltpu.VMEM((2, D, DP), jnp.bfloat16),
            pltpu.VMEM((S, BQ), jnp.float32),
            pltpu.VMEM((S, BQ), jnp.float32),
        ],
        compiler_params=pltpu.CompilerParams(vmem_limit_bytes=110*1024*1024),
    )(A_x.reshape(S, D).T, A_wqkv, A_wo, B_wqkv, B_wo, gate_w.reshape(1, D))
    return out.T.reshape(1, S, D)
```

```python
import functools, math
import jax
import jax.numpy as jnp
import numpy as np
from jax import lax
import jax.experimental.pallas as pl
import jax.experimental.pallas.tpu as pltpu

S, D, H, DH = 2048, 448, 16, 28
HP = 32
DP = H * HP
G = 4 * DH
f32 = jnp.float32; bf16 = jnp.bfloat16
HBM = pltpu.MemorySpace.HBM

def mm(a, b):
    return lax.dot_general(a, b, (((1,), (0,)), ((), ())), preferred_element_type=f32)

def make_kernel(BQ=1024, CK=128, XC=256, OC=256, NITER=None, TIE=2, DMAV=0, LAG=0, CARRY8=True, WBAT=None, GW1D=True, KMODE=0):
    NQ = S // BQ
    NVH = 2 * H
    NT = NVH * NQ
    NC = S // CK
    NX = S // XC
    c_scale = (DH ** -0.5) * math.log2(math.e)

    WP = [(0, 512), (512, 512), (1024, 3*D-1024)]

    def kernel(x_hbm, wqkva_hbm, woa_hbm, wqkvb_hbm, wob_hbm, gw_hbm, o_hbm,
               x_s, wa_s, wb_s, wo_s, gw_s, wt_s, wot_s,
               k_s, qt_s, vt_s, ot_s, g_s, s0_s, s1_s, out_s, sem_in, sem_out):
        cp_x = [pltpu.make_async_copy(x_hbm.at[:, pl.ds(c*XC, XC)], x_s.at[:, pl.ds(c*XC, XC)], sem_in.at[c]) for c in range(NX)]
        cp_wa = [pltpu.make_async_copy(wqkva_hbm.at[:, pl.ds(a, n)], wa_s.at[:, pl.ds(a, n)], sem_in.at[NX+q]) for q, (a, n) in enumerate(WP)]
        cp_gw = pltpu.make_async_copy(gw_hbm, gw_s, sem_in.at[NX+3])
        cp_wb = pltpu.make_async_copy(wqkvb_hbm, wb_s, sem_in.at[NX+4])
        cp_woa = pltpu.make_async_copy(woa_hbm, wo_s.at[pl.ds(0, D), :], sem_in.at[NX+5])
        cp_wob = pltpu.make_async_copy(wob_hbm, wo_s.at[pl.ds(D, D), :], sem_in.at[NX+6])
        cp_wa[0].start(); cp_x[0].start()
        if DMAV == 0:
            cp_wa[1].start(); cp_wa[2].start(); cp_gw.start()
            for c in range(1, NX): cp_x[c].start()
        elif DMAV == 1:
            cp_wa[1].start(); cp_wa[2].start(); cp_gw.start()

        def prep_w(blk, w_ref, a, n):
            wt_s[blk, a:a+n, :] = w_ref[:, a:a+n].T

        def loc(c):
            cs = slice(c*XC, (c+1)*XC)
            i = (c*XC) // BQ
            return cs, i, slice(c*XC - i*BQ, (c+1)*XC - i*BQ)

        zpad = lambda: jnp.zeros((HP-DH, XC), f32)
        def proj_q(blk, c):
            cs, i, qs = loc(c)
            qt = mm(wt_s[blk, 0:D, :], x_s[:, cs]) * c_scale
            for h in range(H):
                blkq = jnp.concatenate([qt[DH*h:DH*(h+1), :], zpad()], axis=0)
                qt_s[(blk*H+h)*NQ + i, :, qs] = blkq.astype(bf16)

        def proj_k(blk, c):
            cs, i, qs = loc(c)
            kt = mm(wt_s[blk, D:2*D, :], x_s[:, cs])
            if KMODE == 0:
                for h in range(H):
                    blkk = jnp.concatenate([kt[DH*h:DH*(h+1), :], zpad()], axis=0)
                    k_s[blk*H+h, cs, :] = blkk.T.astype(bf16)
            else:
                for g in range(4):
                    rows = [kt[DH*h:DH*(h+1), :] for h in range(4*g, 4*g+4)]
                    pieces = []
                    for r_ in rows:
                        pieces += [r_, zpad()]
                    tg = jnp.concatenate(pieces, axis=0).T
                    for j in range(4):
                        sh = tg if j == 0 else pltpu.roll(tg, 128 - HP*j, 1)
                        k_s[blk*H+4*g+j, cs, :] = sh[:, 0:HP].astype(bf16)

        def proj_v(blk, c):
            cs, i, qs = loc(c)
            if blk == 0:
                vt = mm(wt_s[blk, 2*D:3*D+16, :], x_s[:, cs])
                g_s[:, cs] = jnp.broadcast_to(jax.nn.sigmoid(vt[D:D+1, :]), (8, XC))
            else:
                vt = mm(wt_s[blk, 2*D:3*D, :], x_s[:, cs])
            tail = jnp.concatenate([jnp.ones((1, XC), f32), jnp.zeros((HP-DH-1, XC), f32)], axis=0)
            for h in range(H):
                vt_s[blk*H + h, :, cs] = jnp.concatenate([vt[DH*h:DH*(h+1), :], tail], axis=0).astype(bf16)

        def project(blk, c):
            proj_q(blk, c); proj_k(blk, c); proj_v(blk, c)

        cp_wa[0].wait(); cp_x[0].wait()
        if DMAV == 2:
            cp_wa[1].start(); cp_wa[2].start(); cp_gw.start()
        prep_w(0, wa_s, *WP[0])
        proj_q(0, 0)
        cp_wa[1].wait()
        prep_w(0, wa_s, *WP[1])
        proj_k(0, 0)
        cp_wa[2].wait(); cp_gw.wait()
        if DMAV >= 1:
            for c in range(1, NX): cp_x[c].start()
        prep_w(0, wa_s, *WP[2])
        wt_s[0, 3*D:3*D+16, :] = jnp.broadcast_to(gw_s[...].reshape(1, D), (16, D))
        proj_v(0, 0)
        cp_wb.start(); cp_woa.start(); cp_wob.start()
        wb_at = NX - 2 if WBAT is None else WBAT
        for c in range(1, NX):
            cp_x[c].wait()
            if c == wb_at:
                cp_wb.wait()
            if wb_at <= c < wb_at + 3 and WBAT is not None:
                prep_w(1, wb_s, *WP[c - wb_at])
            elif c == wb_at and WBAT is None:
                for (a, n) in WP:
                    prep_w(1, wb_s, a, n)
            project(0, c)
        for c in range(NX):
            if c == NX // 2:
                cp_woa.wait(); cp_wob.wait()
                wot_s[...] = wo_s[...].T
            project(1, c)

        def decode(t):
            return t % NVH, t // NVH

        def qmask(t):
            h, i = decode(t)
            return h, qt_s[h*NQ + i]

        def step(t_cur, s_cur, m_cur, t_nxt, s_nxt):
            macc = None
            o = None
            hist = []
            if t_nxt is not None:
                gidx, qm = qmask(t_nxt)
            if t_cur is not None:
                h, i = decode(t_cur)
            if CARRY8 and t_cur is not None:
                m_cur = jnp.max(m_cur, axis=0, keepdims=True)
            sched = []
            nq_done = 0
            for c in range(NC):
                if t_nxt is not None:
                    upto = min(c + 1, NC - LAG) if t_cur is not None else c + 1
                    while nq_done < upto:
                        sched.append(('qk', nq_done)); nq_done += 1
                if t_cur is not None:
                    sched.append(('pv', c))
            if t_nxt is not None:
                while nq_done < NC:
                    sched.append(('qk', nq_done)); nq_done += 1
            for kind, c in sched:
                sl = slice(c*CK, (c+1)*CK)
                if kind == 'qk':
                    s = mm(k_s[gidx, sl, :], qm)
                    s_nxt[sl, :] = s
                    mx = jnp.max(s.reshape(CK//8, 8, BQ), axis=0)
                    macc = mx if macc is None else jnp.maximum(macc, mx)
                    hist.append(mx)
                else:
                    m_eff = m_cur
                    if len(hist) >= TIE:
                        z = lax.bitcast_convert_type(hist[-TIE][0:1, :], jnp.uint32)
                        z = lax.shift_right_logical(lax.shift_right_logical(z, jnp.uint32(31)), jnp.uint32(1))
                        m_eff = lax.bitcast_convert_type(lax.bitcast_convert_type(m_eff, jnp.uint32) | z, f32)
                    p = jnp.exp2(s_cur[sl, :] - m_eff).astype(bf16)
                    oc = mm(vt_s[h, :, sl], p)
                    o = oc if o is None else o + oc
            on = None
            if t_cur is not None:
                gate = g_s[0:1, pl.ds(pl.multiple_of(i*BQ, BQ), BQ)]
                gate = jnp.where(h < H, gate, 1.0 - gate)
                on = o[0:DH, :] * (gate / o[DH:DH+1, :])
            m_nxt = (macc if CARRY8 else jnp.max(macc, axis=0, keepdims=True)) if t_nxt is not None else None
            return m_nxt, on

        def store_pair(t, on0, on1):
            h, i = decode(t)
            ot_s[i, pl.ds(pl.multiple_of(h*DH, 8), 2*DH), :] = jnp.concatenate([on0, on1], axis=0)

        def out_proj(i):
            for c in range(BQ // OC):
                cs = pl.ds(i*BQ + c*OC, OC)
                y = mm(wot_s[...], ot_s[i, :, c*OC:(c+1)*OC].astype(bf16))
                out_s[:, cs] = y.astype(bf16)
                out_cp(i*(BQ//OC) + c).start()

        def out_cp(n):
            return pltpu.make_async_copy(out_s.at[:, pl.ds(n*OC, OC)], o_hbm.at[:, pl.ds(n*OC, OC)], sem_out.at[n])

        m0, _ = step(None, None, None, 0, s0_s)
        def body(u, m):
            t = 2*u
            m, on0 = step(t, s0_s, m, t+1, s1_s)
            m, on1 = step(t+1, s1_s, m, t+2, s0_s)
            store_pair(t, on0, on1)
            return m
        m = lax.fori_loop(0, NITER or (NT//2 - 1), body, m0)
        m, on0 = step(NT-2, s0_s, m, NT-1, s1_s)
        for i in range(NQ-1):
            out_proj(i)
        _, on1 = step(NT-1, s1_s, m, None, None)
        store_pair(NT-2, on0, on1)
        out_proj(NQ-1)
        for n in range(S // OC):
            out_cp(n).wait()

    scratch = [
        pltpu.VMEM((D, S), bf16),
        pltpu.VMEM((D, 3*D), bf16),
        pltpu.VMEM((D, 3*D), bf16),
        pltpu.VMEM((2*D, D), bf16),
        pltpu.VMEM((D,) if GW1D else (1, D), bf16),
        pltpu.VMEM((2, 3*D+16, D), bf16),
        pltpu.VMEM((D, 2*D), bf16),
        pltpu.VMEM((NVH, S, HP), bf16),
        pltpu.VMEM((NVH*NQ, HP, BQ), bf16),
        pltpu.VMEM((NVH, HP, S), bf16),
        pltpu.VMEM((NQ, 2*D, BQ), f32),
        pltpu.VMEM((8, S), f32),
        pltpu.VMEM((S, BQ), f32),
        pltpu.VMEM((S, BQ), f32),
        pltpu.VMEM((D, S), bf16),
        pltpu.SemaphoreType.DMA((NX+7,)),
        pltpu.SemaphoreType.DMA((S//OC,)),
    ]
    return kernel, scratch


@jax.jit
def pallas_gated_mix__mha_block__softmax_full_mha__prompt_kernel(
    A_x: jax.Array,
    A_wqkv: jax.Array,
    A_wo: jax.Array,
    B_x: jax.Array,
    B_wqkv: jax.Array,
    B_wo: jax.Array,
    gate_w: jax.Array,
):
    del B_x
    kernel, scratch = make_kernel(XC=512)
    out_t = pl.pallas_call(
        kernel,
        out_shape=jax.ShapeDtypeStruct((D, S), jnp.bfloat16),
        in_specs=[pl.BlockSpec(memory_space=HBM)] * 6,
        out_specs=pl.BlockSpec(memory_space=HBM),
        scratch_shapes=scratch,
        compiler_params=pltpu.CompilerParams(vmem_limit_bytes=110 * 1024 * 1024),
    )(A_x.reshape(S, D).T, A_wqkv, A_wo, B_wqkv, B_wo, gate_w)
    return out_t.T.reshape(1, S, D)
```

```python
import math

import jax
import jax.numpy as jnp
from jax import lax
import jax.experimental.pallas as pl
import jax.experimental.pallas.tpu as pltpu

S, D, H, DH = 2048, 448, 16, 28
HP = 32
NVH = 2 * H
BQ = 1024
NQ = S // BQ
NT = NVH * NQ
CK = 128
NC = S // CK
XC = 512
NX = S // XC
OC = 256
UNR = 4
GW_ROWS = 16
W_PIECES = ((0, 512), (512, 512), (1024, 3 * D - 1024))
C_SCALE = (DH ** -0.5) * math.log2(math.e)

f32 = jnp.float32
bf16 = jnp.bfloat16


def _mm(a, b):
    return lax.dot_general(a, b, (((1,), (0,)), ((), ())), preferred_element_type=f32)


def _tie(m, other):
    z = lax.bitcast_convert_type(other, jnp.uint32)
    z = lax.shift_right_logical(lax.shift_right_logical(z, jnp.uint32(31)), jnp.uint32(1))
    return lax.bitcast_convert_type(lax.bitcast_convert_type(m, jnp.uint32) | z, f32)


def _kernel(x_hbm, wqkva_hbm, woa_hbm, wqkvb_hbm, wob_hbm, gw_hbm, o_hbm,
            x_s, wa_s, wb_s, wo_s, gw_s, wt_s, wot_s,
            k_s, qt_s, vt_s, ot_s, g_s, s0_s, s1_s, out_s, sem_in, sem_out):
    cp_x = [pltpu.make_async_copy(x_hbm.at[:, pl.ds(c * XC, XC)], x_s.at[:, pl.ds(c * XC, XC)], sem_in.at[c])
            for c in range(NX)]
    cp_wa = [pltpu.make_async_copy(wqkva_hbm.at[:, pl.ds(a, n)], wa_s.at[:, pl.ds(a, n)], sem_in.at[NX + q])
             for q, (a, n) in enumerate(W_PIECES)]
    cp_gw = pltpu.make_async_copy(gw_hbm, gw_s, sem_in.at[NX + 3])
    cp_wb = pltpu.make_async_copy(wqkvb_hbm, wb_s, sem_in.at[NX + 4])
    cp_woa = pltpu.make_async_copy(woa_hbm, wo_s.at[pl.ds(0, D), :], sem_in.at[NX + 5])
    cp_wob = pltpu.make_async_copy(wob_hbm, wo_s.at[pl.ds(D, D), :], sem_in.at[NX + 6])
    cp_wa[0].start()
    cp_x[0].start()
    cp_wa[1].start()
    cp_wa[2].start()
    cp_gw.start()
    for c in range(1, NX):
        cp_x[c].start()

    def prep_w(blk, w_ref, a, n):
        wt_s[blk, a:a + n, :] = w_ref[:, a:a + n].T

    def loc(c):
        i = (c * XC) // BQ
        return slice(c * XC, (c + 1) * XC), i, slice(c * XC - i * BQ, (c + 1) * XC - i * BQ)

    def zpad():
        return jnp.zeros((HP - DH, XC), f32)

    def proj_q(blk, c):
        cs, i, qs = loc(c)
        qt = _mm(wt_s[blk, 0:D, :], x_s[:, cs]) * C_SCALE
        for h in range(H):
            blkq = jnp.concatenate([qt[DH * h:DH * (h + 1), :], zpad()], axis=0)
            qt_s[(blk * H + h) * NQ + i, :, qs] = blkq.astype(bf16)

    def proj_k(blk, c):
        cs, _, _ = loc(c)
        kt = _mm(wt_s[blk, D:2 * D, :], x_s[:, cs])
        for h in range(H):
            blkk = jnp.concatenate([kt[DH * h:DH * (h + 1), :], zpad()], axis=0)
            k_s[blk * H + h, cs, :] = blkk.T.astype(bf16)

    def proj_v(blk, c):
        cs, _, _ = loc(c)
        if blk == 0:
            vt = _mm(wt_s[blk, 2 * D:3 * D + GW_ROWS, :], x_s[:, cs])
            g_s[:, cs] = jnp.broadcast_to(jax.nn.sigmoid(vt[D:D + 1, :]), (8, XC))
        else:
            vt = _mm(wt_s[blk, 2 * D:3 * D, :], x_s[:, cs])
        tail = jnp.concatenate([jnp.ones((1, XC), f32), jnp.zeros((HP - DH - 1, XC), f32)], axis=0)
        for h in range(H):
            vt_s[blk * H + h, :, cs] = jnp.concatenate([vt[DH * h:DH * (h + 1), :], tail], axis=0).astype(bf16)

    def project(blk, c):
        proj_q(blk, c)
        proj_k(blk, c)
        proj_v(blk, c)

    cp_wa[0].wait()
    cp_x[0].wait()
    prep_w(0, wa_s, *W_PIECES[0])
    proj_q(0, 0)
    cp_wa[1].wait()
    prep_w(0, wa_s, *W_PIECES[1])
    proj_k(0, 0)
    cp_wa[2].wait()
    cp_gw.wait()
    prep_w(0, wa_s, *W_PIECES[2])
    wt_s[0, 3 * D:3 * D + GW_ROWS, :] = jnp.broadcast_to(gw_s[...].reshape(1, D), (GW_ROWS, D))
    proj_v(0, 0)
    cp_wb.start()
    cp_woa.start()
    cp_wob.start()
    for c in range(1, NX):
        cp_x[c].wait()
        if c == NX - 2:
            cp_wb.wait()
            for a, n in W_PIECES:
                prep_w(1, wb_s, a, n)
        project(0, c)
    for c in range(NX):
        if c == NX // 2:
            cp_woa.wait()
            cp_wob.wait()
            wot_s[...] = wo_s[...].T
        project(1, c)

    def decode(t):
        return t % NVH, t // NVH

    def step(t_cur, s_cur, m_cur, t_nxt, s_nxt, filler=None):
        macc = None
        o = None
        hist = []
        if t_nxt is not None:
            hn, i_n = decode(t_nxt)
            qm = qt_s[hn * NQ + i_n]
        if t_cur is not None:
            h, i = decode(t_cur)
            m_cur = jnp.max(m_cur, axis=0, keepdims=True)
        for c in range(NC):
            sl = slice(c * CK, (c + 1) * CK)
            if t_nxt is not None:
                s = _mm(k_s[hn, sl, :], qm)
                s_nxt[sl, :] = s
                mx = jnp.max(s.reshape(CK // 8, 8, BQ), axis=0)
                macc = mx if macc is None else jnp.maximum(macc, mx)
                hist.append(mx)
            if t_cur is not None:
                m_eff = _tie(m_cur, hist[-2][0:1, :]) if len(hist) >= 2 else m_cur
                p = jnp.exp2(s_cur[sl, :] - m_eff).astype(bf16)
                oc = _mm(vt_s[h, :, sl], p)
                o = oc if o is None else o + oc
                if filler is not None:
                    filler(c)
        on = None
        if t_cur is not None:
            gate = g_s[0:1, pl.ds(pl.multiple_of(i * BQ, BQ), BQ)]
            gate = jnp.where(h < H, gate, 1.0 - gate)
            on = o[0:DH, :] * (gate / o[DH:DH + 1, :])
        return macc, on

    def store_pair(t, on0, on1):
        h, i = decode(t)
        ot_s[i, pl.ds(pl.multiple_of(h * DH, 8), 2 * DH), :] = jnp.concatenate([on0, on1], axis=0)

    def pair(t, m):
        m, on0 = step(t, s0_s, m, t + 1, s1_s)
        m, on1 = step(t + 1, s1_s, m, t + 2, s0_s)
        store_pair(t, on0, on1)
        return m

    def body(u, m):
        for e in range(UNR // 2):
            m = pair(UNR * u + 2 * e, m)
        return m

    def out_cp(n):
        return pltpu.make_async_copy(out_s.at[:, pl.ds(n * OC, OC)], o_hbm.at[:, pl.ds(n * OC, OC)], sem_out.at[n])

    def out_chunk(i, c):
        y = _mm(wot_s[...], ot_s[i, :, c * OC:(c + 1) * OC].astype(bf16))
        out_s[:, pl.ds(i * BQ + c * OC, OC)] = y.astype(bf16)
        out_cp(i * (BQ // OC) + c).start()

    m, _ = step(None, None, None, 0, s0_s)
    nit = (NT - 2) // UNR
    m = lax.fori_loop(0, nit, body, m)
    for t in range(nit * UNR, NT - 2, 2):
        m = pair(t, m)
    m, on0 = step(NT - 2, s0_s, m, NT - 1, s1_s)

    todo = [(i, c) for i in range(NQ - 1) for c in range(BQ // OC)]
    done = set()

    def filler(c):
        lo = (len(todo) * (c + 3)) // NC
        hi = min((len(todo) * (c + 4)) // NC, len(todo))
        for n in range(lo, hi):
            if n not in done:
                done.add(n)
                out_chunk(*todo[n])

    _, on1 = step(NT - 1, s1_s, m, None, None, filler)
    for n in range(len(todo)):
        if n not in done:
            out_chunk(*todo[n])
    store_pair(NT - 2, on0, on1)
    for c in range(BQ // OC):
        out_chunk(NQ - 1, c)
    for n in range(S // OC):
        out_cp(n).wait()


@jax.jit
def pallas_gated_mix__mha_block__softmax_full_mha__prompt_kernel(
    A_x: jax.Array,
    A_wqkv: jax.Array,
    A_wo: jax.Array,
    B_x: jax.Array,
    B_wqkv: jax.Array,
    B_wo: jax.Array,
    gate_w: jax.Array,
):
    del B_x
    hbm = pl.BlockSpec(memory_space=pltpu.MemorySpace.HBM)
    out_t = pl.pallas_call(
        _kernel,
        out_shape=jax.ShapeDtypeStruct((D, S), bf16),
        in_specs=[hbm] * 6,
        out_specs=hbm,
        scratch_shapes=[
            pltpu.VMEM((D, S), bf16),
            pltpu.VMEM((D, 3 * D), bf16),
            pltpu.VMEM((D, 3 * D), bf16),
            pltpu.VMEM((2 * D, D), bf16),
            pltpu.VMEM((D,), bf16),
            pltpu.VMEM((2, 3 * D + GW_ROWS, D), bf16),
            pltpu.VMEM((D, 2 * D), bf16),
            pltpu.VMEM((NVH, S, HP), bf16),
            pltpu.VMEM((NVH * NQ, HP, BQ), bf16),
            pltpu.VMEM((NVH, HP, S), bf16),
            pltpu.VMEM((NQ, 2 * D, BQ), f32),
            pltpu.VMEM((8, S), f32),
            pltpu.VMEM((S, BQ), f32),
            pltpu.VMEM((S, BQ), f32),
            pltpu.VMEM((D, S), bf16),
            pltpu.SemaphoreType.DMA((NX + 7,)),
            pltpu.SemaphoreType.DMA((S // OC,)),
        ],
        compiler_params=pltpu.CompilerParams(vmem_limit_bytes=110 * 1024 * 1024),
    )(A_x.reshape(S, D).T, A_wqkv, A_wo, B_wqkv, B_wo, gate_w)
    return out_t.T.reshape(1, S, D)
```

```python
import math

import jax
import jax.numpy as jnp
from jax import lax
import jax.experimental.pallas as pl
import jax.experimental.pallas.tpu as pltpu

S, D, H, DH = 2048, 448, 16, 28
HP = 32
NVH = 2 * H
BQ = 1024
NQ = S // BQ
NT = NVH * NQ
CK = 128
NC = S // CK
XC = 512
NX = S // XC
OC = 256
UNR = 4
GW_ROWS = 16
W_PIECES = ((0, 512), (512, 512), (1024, 3 * D - 1024))
C_SCALE = (DH ** -0.5) * math.log2(math.e)

f32 = jnp.float32
bf16 = jnp.bfloat16


def _mm(a, b):
    return lax.dot_general(a, b, (((1,), (0,)), ((), ())), preferred_element_type=f32)


def _tie(m, other):
    z = lax.bitcast_convert_type(other, jnp.uint32)
    z = lax.shift_right_logical(lax.shift_right_logical(z, jnp.uint32(31)), jnp.uint32(1))
    return lax.bitcast_convert_type(lax.bitcast_convert_type(m, jnp.uint32) | z, f32)


def _kernel(x_hbm, wqkva_hbm, woa_hbm, wqkvb_hbm, wob_hbm, gw_hbm, o_hbm,
            x_s, wa_s, wb_s, wo_s, gw_s, wt_s, wot_s,
            k_s, qt_s, vt_s, ot_s, g_s, s0_s, s1_s, out_s, sem_in, sem_out):
    cp_x = [pltpu.make_async_copy(x_hbm.at[:, pl.ds(c * XC, XC)], x_s.at[:, pl.ds(c * XC, XC)], sem_in.at[c])
            for c in range(NX)]
    cp_wa = [pltpu.make_async_copy(wqkva_hbm.at[:, pl.ds(a, n)], wa_s.at[:, pl.ds(a, n)], sem_in.at[NX + q])
             for q, (a, n) in enumerate(W_PIECES)]
    cp_gw = pltpu.make_async_copy(gw_hbm, gw_s, sem_in.at[NX + 3])
    cp_wb = pltpu.make_async_copy(wqkvb_hbm, wb_s, sem_in.at[NX + 4])
    cp_woa = pltpu.make_async_copy(woa_hbm, wo_s.at[pl.ds(0, D), :], sem_in.at[NX + 5])
    cp_wob = pltpu.make_async_copy(wob_hbm, wo_s.at[pl.ds(D, D), :], sem_in.at[NX + 6])
    cp_wa[0].start()
    cp_x[0].start()
    cp_wa[1].start()
    cp_wa[2].start()
    cp_gw.start()
    for c in range(1, NX):
        cp_x[c].start()

    def prep_w(blk, w_ref, a, n):
        wt_s[blk, a:a + n, :] = w_ref[:, a:a + n].T

    def loc(c):
        i = (c * XC) // BQ
        return slice(c * XC, (c + 1) * XC), i, slice(c * XC - i * BQ, (c + 1) * XC - i * BQ)

    def zpad():
        return jnp.zeros((HP - DH, XC), f32)

    def proj_q(blk, c):
        cs, i, qs = loc(c)
        qt = _mm(wt_s[blk, 0:D, :], x_s[:, cs]) * C_SCALE
        for h in range(H):
            blkq = jnp.concatenate([qt[DH * h:DH * (h + 1), :], zpad()], axis=0)
            qt_s[(blk * H + h) * NQ + i, :, qs] = blkq.astype(bf16)

    def proj_k(blk, c):
        cs, _, _ = loc(c)
        kt = _mm(wt_s[blk, D:2 * D, :], x_s[:, cs])
        for h in range(H):
            blkk = jnp.concatenate([kt[DH * h:DH * (h + 1), :], zpad()], axis=0)
            k_s[blk * H + h, cs, :] = blkk.T.astype(bf16)

    def proj_v(blk, c):
        cs, _, _ = loc(c)
        if blk == 0:
            vt = _mm(wt_s[blk, 2 * D:3 * D + GW_ROWS, :], x_s[:, cs])
            g_s[:, cs] = jnp.broadcast_to(jax.nn.sigmoid(vt[D:D + 1, :]), (8, XC))
        else:
            vt = _mm(wt_s[blk, 2 * D:3 * D, :], x_s[:, cs])
        tail = jnp.concatenate([jnp.ones((1, XC), f32), jnp.zeros((HP - DH - 1, XC), f32)], axis=0)
        for h in range(H):
            vt_s[blk * H + h, :, cs] = jnp.concatenate([vt[DH * h:DH * (h + 1), :], tail], axis=0).astype(bf16)

    def project(blk, c):
        proj_q(blk, c)
        proj_k(blk, c)
        proj_v(blk, c)

    cp_wa[0].wait()
    cp_x[0].wait()
    prep_w(0, wa_s, *W_PIECES[0])
    proj_q(0, 0)
    cp_wa[1].wait()
    prep_w(0, wa_s, *W_PIECES[1])
    proj_k(0, 0)
    cp_wa[2].wait()
    cp_gw.wait()
    prep_w(0, wa_s, *W_PIECES[2])
    wt_s[0, 3 * D:3 * D + GW_ROWS, :] = jnp.broadcast_to(gw_s[...].reshape(1, D), (GW_ROWS, D))
    proj_v(0, 0)
    cp_wb.start()
    cp_woa.start()
    cp_wob.start()
    for c in range(1, NX):
        cp_x[c].wait()
        if c == NX - 2:
            cp_wb.wait()
            for a, n in W_PIECES:
                prep_w(1, wb_s, a, n)
        project(0, c)
    for c in range(NX):
        project(1, c)

    def decode(t):
        return t % NVH, t // NVH

    def step(t_cur, s_cur, m_cur, t_nxt, s_nxt, filler=None):
        macc = None
        o = None
        hist = []
        if t_nxt is not None:
            hn, i_n = decode(t_nxt)
            qm = qt_s[hn * NQ + i_n]
        if t_cur is not None:
            h, i = decode(t_cur)
            m_cur = jnp.max(m_cur, axis=0, keepdims=True)
        for c in range(NC):
            sl = slice(c * CK, (c + 1) * CK)
            if t_nxt is not None:
                s = _mm(k_s[hn, sl, :], qm)
                s_nxt[sl, :] = s
                mx = jnp.max(s.reshape(CK // 8, 8, BQ), axis=0)
                macc = mx if macc is None else jnp.maximum(macc, mx)
                hist.append(mx)
            if t_cur is not None:
                m_eff = _tie(m_cur, hist[-2][0:1, :]) if len(hist) >= 2 else m_cur
                p = jnp.exp2(s_cur[sl, :] - m_eff).astype(bf16)
                oc = _mm(vt_s[h, :, sl], p)
                o = oc if o is None else o + oc
                if filler is not None:
                    filler(c)
        on = None
        if t_cur is not None:
            gate = g_s[0:1, pl.ds(pl.multiple_of(i * BQ, BQ), BQ)]
            gate = jnp.where(h < H, gate, 1.0 - gate)
            on = o[0:DH, :] * (gate / o[DH:DH + 1, :])
        return macc, on

    def store_pair(t, on0, on1):
        h, i = decode(t)
        ot_s[i, pl.ds(pl.multiple_of(h * DH, 8), 2 * DH), :] = jnp.concatenate([on0, on1], axis=0)

    def pair(t, m):
        m, on0 = step(t, s0_s, m, t + 1, s1_s)
        m, on1 = step(t + 1, s1_s, m, t + 2, s0_s)
        store_pair(t, on0, on1)
        return m

    def body(u, m):
        for e in range(UNR // 2):
            m = pair(UNR * u + 2 * e, m)
        return m

    def out_cp(n):
        return pltpu.make_async_copy(out_s.at[:, pl.ds(n * OC, OC)], o_hbm.at[:, pl.ds(n * OC, OC)], sem_out.at[n])

    def out_chunk(i, c):
        y = _mm(wot_s[...], ot_s[i, :, c * OC:(c + 1) * OC].astype(bf16))
        out_s[:, pl.ds(i * BQ + c * OC, OC)] = y.astype(bf16)
        out_cp(i * (BQ // OC) + c).start()

    m, _ = step(None, None, None, 0, s0_s)
    nit = (NT - 2) // UNR
    m = lax.fori_loop(0, nit, body, m)
    cp_woa.wait()
    cp_wob.wait()
    wot_s[...] = wo_s[...].T
    for t in range(nit * UNR, NT - 2, 2):
        m = pair(t, m)
    m, on0 = step(NT - 2, s0_s, m, NT - 1, s1_s)

    todo = [(i, c) for i in range(NQ - 1) for c in range(BQ // OC)]
    done = set()

    def filler(c):
        lo = (len(todo) * (c + 3)) // NC
        hi = min((len(todo) * (c + 4)) // NC, len(todo))
        for n in range(lo, hi):
            if n not in done:
                done.add(n)
                out_chunk(*todo[n])

    _, on1 = step(NT - 1, s1_s, m, None, None, filler)
    for n in range(len(todo)):
        if n not in done:
            out_chunk(*todo[n])
    store_pair(NT - 2, on0, on1)
    for c in range(BQ // OC):
        out_chunk(NQ - 1, c)
    for n in range(S // OC):
        out_cp(n).wait()


@jax.jit
def pallas_gated_mix__mha_block__softmax_full_mha__prompt_kernel(
    A_x: jax.Array,
    A_wqkv: jax.Array,
    A_wo: jax.Array,
    B_x: jax.Array,
    B_wqkv: jax.Array,
    B_wo: jax.Array,
    gate_w: jax.Array,
):
    del B_x
    hbm = pl.BlockSpec(memory_space=pltpu.MemorySpace.HBM)
    out_t = pl.pallas_call(
        _kernel,
        out_shape=jax.ShapeDtypeStruct((D, S), bf16),
        in_specs=[hbm] * 6,
        out_specs=hbm,
        scratch_shapes=[
            pltpu.VMEM((D, S), bf16),
            pltpu.VMEM((D, 3 * D), bf16),
            pltpu.VMEM((D, 3 * D), bf16),
            pltpu.VMEM((2 * D, D), bf16),
            pltpu.VMEM((D,), bf16),
            pltpu.VMEM((2, 3 * D + GW_ROWS, D), bf16),
            pltpu.VMEM((D, 2 * D), bf16),
            pltpu.VMEM((NVH, S, HP), bf16),
            pltpu.VMEM((NVH * NQ, HP, BQ), bf16),
            pltpu.VMEM((NVH, HP, S), bf16),
            pltpu.VMEM((NQ, 2 * D, BQ), f32),
            pltpu.VMEM((8, S), f32),
            pltpu.VMEM((S, BQ), f32),
            pltpu.VMEM((S, BQ), f32),
            pltpu.VMEM((D, S), bf16),
            pltpu.SemaphoreType.DMA((NX + 7,)),
            pltpu.SemaphoreType.DMA((S // OC,)),
        ],
        compiler_params=pltpu.CompilerParams(vmem_limit_bytes=110 * 1024 * 1024),
    )(A_x.reshape(S, D).T, A_wqkv, A_wo, B_wqkv, B_wo, gate_w)
    return out_t.T.reshape(1, S, D)
```
